```python
import os as _os
_os.environ.setdefault("JAX_PLATFORMS", "cpu")
import jax
import jax.numpy as jnp

def _softmax(x, axis=-1):
    return jax.nn.softmax(x, axis=axis)
def _gelu(x):
    return jax.nn.gelu(x, approximate=True)
def _silu(x):
    return jax.nn.silu(x)
def _sigmoid(x):
    return jax.nn.sigmoid(x)
def _layernorm(x, axis=-1, eps=1e-5):
    m = jnp.mean(x, axis=axis, keepdims=True)
    v = jnp.var(x, axis=axis, keepdims=True)
    return (x - m) / jnp.sqrt(v + eps)
def _scatter_add(tgt, idx, src, axis=0):
    return tgt.at[idx].add(src)
def _segment_sum(src, seg, n):
    return jax.ops.segment_sum(src, seg, n)
class _Rng:
    def __init__(self, key):
        self._k = key
    def _next(self):
        self._k, sub = jax.random.split(self._k)
        return sub
    def normal(self, shape):
        return jax.random.normal(self._next(), shape, dtype=jnp.bfloat16)
    def randint(self, lo, hi, shape):
        return jax.random.randint(self._next(), shape, lo, hi, dtype=jnp.int32)
    def uniform(self, shape, lo=0.0, hi=1.0):
        return jax.random.uniform(self._next(), shape, jnp.bfloat16, lo, hi)
    def permutation(self, n):
        return jax.random.permutation(self._next(), n)


kernel_name = 'concat_heads__linear_kernel_hedgehog__ssm_conv_s5__prompt'

def setup_inputs():
    _rng = _Rng(jax.random.key(int.from_bytes(__import__("os").urandom(4), "little")))
    _w = (lambda a: (lambda t: t.astype(jnp.bfloat16) if jnp.issubdtype(t.dtype, jnp.floating) else t)(jnp.asarray(a)))
    def _A_setup():
        B, S, D, H = 1, 2048, 640, 32
        Dh = D // H
        return {
            "x": _w((lambda *s: _rng.normal(s) * 0.4)(B, S, D)),
            "wqkv": _w((lambda *s: _rng.normal(s) * 0.4)(D, 3 * D)),
            "w_phi": _w((lambda *s: _rng.normal(s) * 0.4)(H, Dh, Dh) * (Dh ** -0.5)),
            "wo": _w((lambda *s: _rng.normal(s) * 0.05)(D, D)),
        }
    _A_in = _A_setup()

    def _B_setup():
        B, S, D = 1, 2048, 640
        P = D
        Lambda_re = -0.5 * jnp.exp((lambda *s: _rng.normal(s) * 0.8)(P))
        Lambda_im = (lambda *s: _rng.normal(s) * 0.8)(P) * 1.0
        B_re = (lambda *s: _rng.normal(s) * 0.8)(P, D) * (D ** -0.5)
        B_im = (lambda *s: _rng.normal(s) * 0.8)(P, D) * (D ** -0.5)
        C_re = (lambda *s: _rng.normal(s) * 0.8)(D, P) * (P ** -0.5)
        C_im = (lambda *s: _rng.normal(s) * 0.8)(D, P) * (P ** -0.5)
        log_dt = (lambda *s: _rng.normal(s) * 0.8)(P) * 0.3 - 2.0
        Dskip = (lambda *s: _rng.normal(s) * 0.8)(D)
        return {
            "x": _w((lambda *s: _rng.normal(s) * 0.05)(B, S, D)),
            "Lambda_re": _w(Lambda_re),
            "Lambda_im": _w(Lambda_im),
            "B_re": _w(B_re),
            "B_im": _w(B_im),
            "C_re": _w(C_re),
            "C_im": _w(C_im),
            "log_dt": _w(log_dt),
            "Dskip": _w(Dskip),
        }
    _B_in = _B_setup()

    return {
        "A_x": _A_in["x"],
        "A_wqkv": _A_in["wqkv"],
        "A_w_phi": _A_in["w_phi"],
        "A_wo": _A_in["wo"],
        "B_x": _B_in["x"],
        "B_Lambda_re": _B_in["Lambda_re"],
        "B_Lambda_im": _B_in["Lambda_im"],
        "B_B_re": _B_in["B_re"],
        "B_B_im": _B_in["B_im"],
        "B_C_re": _B_in["C_re"],
        "B_C_im": _B_in["C_im"],
        "B_log_dt": _B_in["log_dt"],
        "B_Dskip": _B_in["Dskip"],
    }

def reference(A_x, A_wqkv, A_w_phi, A_wo, B_x, B_Lambda_re, B_Lambda_im, B_B_re, B_B_im, B_C_re, B_C_im, B_log_dt, B_Dskip):
    def _A_ref(x, wqkv, w_phi, wo):
        B, S, D = x.shape
        H = 32; Dh = D // H
        qkv = (lambda x, *d: x.transpose(*d))((x @ wqkv).reshape(B, S, 3, H, Dh), 2, 0, 3, 1, 4)
        q, k, v = qkv[0], qkv[1], qkv[2]
        pq = jnp.einsum("bhsd,hdf->bhsf", q, w_phi)
        pk = jnp.einsum("bhsd,hdf->bhsf", k, w_phi)
        phi_q = jnp.concatenate([_softmax(pq, axis=-1), _softmax(-pq, axis=-1)], axis=-1)
        phi_k = jnp.concatenate([_softmax(pk, axis=-1), _softmax(-pk, axis=-1)], axis=-1)
        kv = jnp.einsum("bhsf,bhsd->bhfd", phi_k, v)
        z  = jnp.einsum("bhsf->bhf", phi_k)
        num = jnp.einsum("bhqf,bhfd->bhqd", phi_q, kv)
        den = jnp.einsum("bhqf,bhf->bhq", phi_q, z)[..., None] + 1e-6
        o = num / den
        return (lambda x, *d: x.transpose(*d))(o, 0, 2, 1, 3).reshape(B, S, D) @ wo

    def _B_ref(x, Lambda_re, Lambda_im, B_re, B_im, C_re, C_im, log_dt, Dskip):
        Bsz, L, H = x.shape
        Lam = Lambda_re + 1j * Lambda_im
        Bmat = B_re + 1j * B_im
        Cmat = C_re + 1j * C_im
        dt = jnp.exp(log_dt)
        Lam_bar = jnp.exp(dt * Lam)
        B_bar = ((Lam_bar - 1.0) / Lam)[:, None] * Bmat
        Bu = jnp.einsum("bld,pd->blp", x + 0j, B_bar)
        h = jnp.zeros_like(Bu[:, 0, :])
        hs = []
        for t in range(L):
            h = Lam_bar[None, :] * h + Bu[:, t, :]
            hs.append(h)
        hseq = jnp.stack(hs, 1)
        y = 2.0 * jnp.einsum("blp,dp->bld", hseq, Cmat).real + x * Dskip[None, None, :]
        return y

    a = _A_ref(A_x, A_wqkv, A_w_phi, A_wo)
    b = _B_ref(B_x, B_Lambda_re, B_Lambda_im, B_B_re, B_B_im, B_C_re, B_C_im, B_log_dt, B_Dskip)
    return jnp.concatenate([a, b], axis=-1)
```

```python
import functools
import numpy as np
import jax
import jax.numpy as jnp
from jax import lax
import jax.experimental.pallas as pl
import jax.experimental.pallas.tpu as pltpu

SEQ, D, H, DH = 2048, 640, 32, 20
NG = H // 2
GR = 2 * DH
NC = D // 128
LOG2E = float(np.log2(np.e))
F32, BF16 = jnp.float32, jnp.bfloat16
NT = (((1,), (1,)), ((), ()))
TN = (((0,), (0,)), ((), ()))


def _rcp(x):
    r = pltpu.reciprocal(x, approx=True)
    return r * (2.0 - x * r)


def _fdiv(x, n):
    return jnp.floor((x + 0.5) * (1.0 / n))


def _iota(shape, d):
    return lax.broadcasted_iota(jnp.int32, shape, d).astype(F32)


def _dual_softmax(p):
    pj = [p[8 * j:8 * j + 8] for j in range(5)]

    def allred(xs, op):
        m = op(op(op(xs[0], xs[1]), op(xs[2], xs[3])), xs[4])
        m = op(m, pltpu.roll(m, 4, 0))
        return op(m, pltpu.roll(m, 2, 0))

    mx = allred(pj, jnp.maximum)
    mn = allred(pj, jnp.minimum)
    ep = [jnp.exp2(x - mx) for x in pj]
    en = [jnp.exp2(mn - x) for x in pj]
    rp = _rcp(allred(ep, jnp.add))
    rn = _rcp(allred(en, jnp.add))
    return jnp.concatenate([e * rp for e in ep] + [e * rn for e in en], axis=0).astype(BF16)


def _make_kernel(T1, T2):
    N1, N2 = SEQ // T1, SEQ // T2
    TS = T2 + 4

    def kernel(ax_hbm, wqkv_hbm, wphi_hbm, wo_hbm, bx_hbm, lre_hbm, lim_hbm, bre_hbm, bim_hbm,
               cre_hbm, cim_hbm, ldt_hbm, dsk_hbm, out_hbm,
               xa, xb, wq, wk, wv, wo, bre, bim, cre, cim, wphi, lre, lim, ldt, dsk,
               r_scr, m_scr, wkvT, wqT, c2, kvacc, kvm, ur, ui, hr, hi, out_scr,
               sem_w, sem_xa, sem_xb, sem_oa, sem_ob):
        def cp_w(src, dst, k):
            return pltpu.make_async_copy(src, dst, sem_w.at[k])

        def cp_xa(i):
            return pltpu.make_async_copy(ax_hbm.at[pl.ds(i * T1, T1), :], xa.at[pl.ds(i * T1, T1), :], sem_xa.at[i])

        def cp_xb(i):
            return pltpu.make_async_copy(bx_hbm.at[pl.ds(i * T2, T2), :], xb.at[pl.ds(i * T2, T2), :], sem_xb.at[i])

        def cp_oa(i):
            return pltpu.make_async_copy(out_scr.at[pl.ds(i * T2, T2), pl.ds(0, D)],
                                         out_hbm.at[pl.ds(i * T2, T2), pl.ds(0, D)], sem_oa.at[i])

        def cp_ob(i):
            return pltpu.make_async_copy(out_scr.at[pl.ds(i * T2, T2), pl.ds(D, D)],
                                         out_hbm.at[pl.ds(i * T2, T2), pl.ds(D, D)], sem_ob.at[i])

        c_wphi = cp_w(wphi_hbm, wphi, 0)
        c_wk = cp_w(wqkv_hbm.at[:, pl.ds(D, D)], wk, 1)
        c_wv = cp_w(wqkv_hbm.at[:, pl.ds(2 * D, D)], wv, 2)
        c_wq = cp_w(wqkv_hbm.at[:, pl.ds(0, D)], wq, 3)
        c_lre = cp_w(lre_hbm, lre, 4)
        c_lim = cp_w(lim_hbm, lim, 5)
        c_ldt = cp_w(ldt_hbm, ldt, 6)
        c_dsk = cp_w(dsk_hbm, dsk, 7)
        c_cre = cp_w(cre_hbm, cre, 8)
        c_cim = cp_w(cim_hbm, cim, 9)
        c_bre = cp_w(bre_hbm, bre, 10)
        c_bim = cp_w(bim_hbm, bim, 11)
        c_wo = cp_w(wo_hbm, wo, 12)

        c_wphi.start()
        c_wk.start()
        cp_xa(0).start()
        c_wv.start()
        c_lre.start(); c_lim.start(); c_ldt.start(); c_dsk.start()

        c_wphi.wait()
        for h in range(H):
            r_scr[pl.ds(DH * h, DH), :] = wphi[h].astype(F32)
        rr = _iota((160, DH), 0)
        e_t = (_fdiv(rr - 40.0 * _fdiv(rr, 40), 2) == _iota((160, DH), 1)).astype(BF16)
        rr = _iota((160, 128), 0)
        hrow = 2.0 * _fdiv(rr, 40) + (rr - 2.0 * _fdiv(rr, 2))
        cc = _iota((160, 128), 1)
        for j in range(NC):
            rj = r_scr[pl.ds(128 * j, 128), :].astype(BF16)
            full = lax.dot_general(e_t, rj, NT, preferred_element_type=F32)
            mask = (hrow + 6.0 * j) == _fdiv(cc + 128.0 * j, DH)
            m_scr[j] = jnp.where(mask, full, 0.0).astype(BF16)

        def fold_rows(w_ref):
            blks = [lax.dot_general(m_scr[j], w_ref[:, pl.ds(128 * j, 128)], NT, preferred_element_type=F32)
                    for j in range(NC)]
            parts = [blks[0][0:120]]
            for j in range(1, NC):
                parts.append(blks[j - 1][120:160] + blks[j][0:40])
                parts.append(blks[j][40:120])
            parts.append(blks[NC - 1][120:160])
            return (jnp.concatenate(parts, axis=0) * LOG2E).astype(BF16)

        c_wk.wait()
        wkvT[pl.ds(0, D), :] = fold_rows(wk)
        c_wv.wait()
        wkvT[pl.ds(D, D), :] = wv[...].T
        kvacc[...] = jnp.zeros(kvacc.shape, F32)

        c_wq.start()
        c_cre.start(); c_cim.start()
        for i in range(1, N1):
            cp_xa(i).start()
        c_bre.start(); c_bim.start(); c_wo.start()
        for i in range(N2):
            cp_xb(i).start()

        def phase1(i, carry):
            cp_xa(i).wait()
            x = xa[pl.ds(pl.multiple_of(i * T1, T1), T1), :]
            kvT = lax.dot_general(wkvT[...], x, NT, preferred_element_type=F32)
            ones = jnp.ones((8, T1), F32)
            for g in range(NG):
                phi = _dual_softmax(kvT[GR * g:GR * g + GR])
                vext = jnp.concatenate([kvT[D + GR * g:D + GR * g + GR], ones], axis=0).astype(BF16)
                kvacc[g] += lax.dot_general(vext, phi, NT, preferred_element_type=F32)
            return carry

        lax.fori_loop(0, N1, phase1, 0)

        r48 = _iota((48, 2 * GR), 0)
        c80 = _iota((48, 2 * GR), 1)
        head_r = jnp.where(r48 < 40.0, _fdiv(r48, DH), _fdiv(r48 - 40.0, 4))
        kvmask = head_r == (c80 - 2.0 * _fdiv(c80, 2))
        for g in range(NG):
            kvm[g] = jnp.where(kvmask, kvacc[g], 0.0).astype(BF16)

        c_wq.wait()
        wqT[...] = fold_rows(wq)

        c_lre.wait(); c_lim.wait(); c_ldt.wait(); c_dsk.wait()
        l_re = lre[...].astype(F32).reshape(1, D)
        l_im = lim[...].astype(F32).reshape(1, D)
        dt = jnp.exp(ldt[...].astype(F32).reshape(1, D)).astype(BF16).astype(F32)
        mag = jnp.exp(dt * l_re)
        ang = dt * l_im
        lb_re, lb_im = mag * jnp.cos(ang), mag * jnp.sin(ang)
        inv = 1.0 / (l_re * l_re + l_im * l_im)
        nr = lb_re - 1.0
        co_re = 2.0 * (nr * l_re + lb_im * l_im) * inv
        co_im = 2.0 * (lb_im * l_re - nr * l_im) * inv
        c_cre.wait(); c_cim.wait()
        cr, ci = cre[...].astype(F32), cim[...].astype(F32)
        c2[:, pl.ds(0, D)] = (cr * co_re - ci * co_im).astype(BF16)
        c2[:, pl.ds(D, D)] = (-(cr * co_im + ci * co_re)).astype(BF16)
        lam_r = jnp.concatenate([lb_re[:, 128 * c:128 * c + 128] for c in range(NC)], axis=0)
        lam_i = jnp.concatenate([lb_im[:, 128 * c:128 * c + 128] for c in range(NC)], axis=0)
        dskip = dsk[...].astype(F32).reshape(1, D)
        c_bre.wait(); c_bim.wait(); c_wo.wait()

        def phase2(i, carry):
            s_re, s_im = carry
            cp_xb(i).wait()
            r0 = pl.multiple_of(i * T2, T2)
            x_b = xb[pl.ds(r0, T2), :]
            u_re = lax.dot_general(x_b, bre[...], NT, preferred_element_type=F32)
            u_im = lax.dot_general(x_b, bim[...], NT, preferred_element_type=F32)
            for c in range(NC):
                ur[pl.ds(c * TS, T2), :] = u_re[:, 128 * c:128 * c + 128]
                ui[pl.ds(c * TS, T2), :] = u_im[:, 128 * c:128 * c + 128]
            x_a = xa[pl.ds(r0, T2), :]
            pq = lax.dot_general(wqT[...], x_a, NT, preferred_element_type=F32)
            for t in range(T2):
                a = ur[pl.ds(t, NC, stride=TS), :]
                b = ui[pl.ds(t, NC, stride=TS), :]
                s_re, s_im = (lam_r * s_re - lam_i * s_im + a, lam_r * s_im + lam_i * s_re + b)
                hr[pl.ds(t, NC, stride=TS), :] = s_re
                hi[pl.ds(t, NC, stride=TS), :] = s_im
            h_re = jnp.concatenate([hr[pl.ds(c * TS, T2), :] for c in range(NC)], axis=1).astype(BF16)
            h_im = jnp.concatenate([hi[pl.ds(c * TS, T2), :] for c in range(NC)], axis=1).astype(BF16)
            y = lax.dot_general(h_re, c2[:, pl.ds(0, D)], NT, preferred_element_type=F32)
            y = y + lax.dot_general(h_im, c2[:, pl.ds(D, D)], NT, preferred_element_type=F32)
            out_scr[pl.ds(r0, T2), pl.ds(D, D)] = y + x_b.astype(F32) * dskip
            cp_ob(i).start()

            low = lax.broadcasted_iota(jnp.int32, (8, T2), 0) < 4
            outs = []
            for g in range(NG):
                phi = _dual_softmax(pq[GR * g:GR * g + GR])
                nd = jnp.dot(kvm[g], phi, preferred_element_type=F32)
                r = _rcp(nd[40:48] + 1e-6)
                rs = pltpu.roll(r, 4, 0)
                ra, rb = jnp.where(low, r, rs), jnp.where(low, rs, r)
                outs += [nd[0:8] * ra, nd[8:16] * ra, nd[16:24] * r, nd[24:32] * rb, nd[32:40] * rb]
            o_t = jnp.concatenate(outs, axis=0).astype(BF16)
            a_out = lax.dot_general(o_t, wo[...], TN, preferred_element_type=F32)
            out_scr[pl.ds(r0, T2), pl.ds(0, D)] = a_out
            cp_oa(i).start()
            return s_re, s_im

        z = jnp.zeros((NC, 128), F32)
        lax.fori_loop(0, N2, phase2, (z, z))
        for i in range(N2):
            cp_oa(i).wait()
            cp_ob(i).wait()

    return kernel, N1, N2, TS


@jax.jit
def pallas_concat_heads__linear_kernel_hedgehog__ssm_conv_s5__prompt_kernel(
    A_x: jax.Array,
    A_wqkv: jax.Array,
    A_w_phi: jax.Array,
    A_wo: jax.Array,
    B_x: jax.Array,
    B_Lambda_re: jax.Array,
    B_Lambda_im: jax.Array,
    B_B_re: jax.Array,
    B_B_im: jax.Array,
    B_C_re: jax.Array,
    B_C_im: jax.Array,
    B_log_dt: jax.Array,
    B_Dskip: jax.Array,
):
    T1 = 512
    T2 = 512
    kernel, N1, N2, TS = _make_kernel(T1, T2)
    any_spec = pl.BlockSpec(memory_space=pl.ANY)
    V = pltpu.VMEM
    scratch = [
        V((SEQ, D), BF16), V((SEQ, D), BF16),
        V((D, D), BF16), V((D, D), BF16), V((D, D), BF16), V((D, D), BF16),
        V((D, D), BF16), V((D, D), BF16), V((D, D), BF16), V((D, D), BF16),
        V((H, DH, DH), BF16), V((D,), BF16), V((D,), BF16), V((D,), BF16), V((D,), BF16),
        V((D, DH), F32), V((NC, 160, 128), BF16), V((2 * D, D), BF16), V((D, D), BF16), V((D, 2 * D), BF16),
        V((NG, 48, 2 * GR), F32), V((NG, 48, 2 * GR), BF16),
        V((NC * TS + 4, 128), F32), V((NC * TS + 4, 128), F32),
        V((NC * TS + 4, 128), F32), V((NC * TS + 4, 128), F32),
        V((SEQ, 2 * D), F32),
        pltpu.SemaphoreType.DMA((13,)), pltpu.SemaphoreType.DMA((N1,)), pltpu.SemaphoreType.DMA((N2,)),
        pltpu.SemaphoreType.DMA((N2,)), pltpu.SemaphoreType.DMA((N2,)),
    ]
    out = pl.pallas_call(
        kernel,
        out_shape=jax.ShapeDtypeStruct((SEQ, 2 * D), F32),
        in_specs=[any_spec] * 13,
        out_specs=any_spec,
        scratch_shapes=scratch,
        compiler_params=pltpu.CompilerParams(vmem_limit_bytes=100 * 1024 * 1024),
        name="hedgehog_s5",
    )(A_x.reshape(SEQ, D), A_wqkv, A_w_phi, A_wo, B_x.reshape(SEQ, D), B_Lambda_re, B_Lambda_im,
      B_B_re, B_B_im, B_C_re, B_C_im, B_log_dt, B_Dskip)
    return out.reshape(1, SEQ, 2 * D)
```

```python
import numpy as np
import jax
import jax.numpy as jnp
from jax import lax
import jax.experimental.pallas as pl
import jax.experimental.pallas.tpu as pltpu

SEQ, D, H, DH = 2048, 640, 32, 20
NG = H // 2
GR = 2 * DH
NC = D // 128
LOG2E = float(np.log2(np.e))
F32, BF16 = jnp.float32, jnp.bfloat16
NT = (((1,), (1,)), ((), ()))
TN = (((0,), (0,)), ((), ()))


def _mo(v, n):
    return v if isinstance(v, int) else pl.multiple_of(v, n)


def _rcp(x):
    r = pltpu.reciprocal(x, approx=True)
    return r * (2.0 - x * r)


def _fdiv(x, n):
    return jnp.floor((x + 0.5) * (1.0 / n))


def _iota(shape, d):
    return lax.broadcasted_iota(jnp.int32, shape, d).astype(F32)


def _dual_softmax(p):
    pj = [p[8 * j:8 * j + 8] for j in range(5)]

    def allred(xs, op):
        m = op(op(op(xs[0], xs[1]), op(xs[2], xs[3])), xs[4])
        m = op(m, pltpu.roll(m, 4, 0))
        return op(m, pltpu.roll(m, 2, 0))

    mx = allred(pj, jnp.maximum)
    mn = allred(pj, jnp.minimum)
    ep = [jnp.exp2(x - mx) for x in pj]
    en = [jnp.exp2(mn - x) for x in pj]
    rp = _rcp(allred(ep, jnp.add))
    rn = _rcp(allred(en, jnp.add))
    return jnp.concatenate([e * rp for e in ep] + [e * rn for e in en], axis=0).astype(BF16)


def _make_kernel(T1, T2, ORDER, SPLIT_A, SPLIT_B, XFIRST, YROWS, SCOPES):
    N1, N2 = SEQ // T1, SEQ // T2
    TS = T2 + 4
    TSH = T2 // 2 + 4

    def kernel(ax_hbm, wqkv_hbm, wphi_hbm, wo_hbm, bx_hbm, lre_hbm, lim_hbm, bre_hbm, bim_hbm,
               cre_hbm, cim_hbm, ldt_hbm, dsk_hbm, out_hbm,
               xa, xb, wq, wkv, wo, bre, bim, cre, cim, wphi, lre, lim, ldt, dsk,
               r_scr, m_scr, wkT, wvT, wqT, kvacc, kvm, coef, lam, ur, ui, hr, hi, out_scr,
               sem_w, sem_xa, sem_xb, sem_oa, sem_ob):
        scopes = []

        def scope(name):
            if SCOPES:
                if scopes:
                    scopes.pop().__exit__(None, None, None)
                if name:
                    sc = jax.named_scope(name)
                    sc.__enter__()
                    scopes.append(sc)

        def cp_w(src, dst, k):
            return pltpu.make_async_copy(src, dst, sem_w.at[k])

        def cp_xa(i):
            return pltpu.make_async_copy(ax_hbm.at[pl.ds(i * T1, T1), :], xa.at[pl.ds(i * T1, T1), :], sem_xa.at[i])

        def cp_xb(i):
            return pltpu.make_async_copy(bx_hbm.at[pl.ds(i * T2, T2), :], xb.at[pl.ds(i * T2, T2), :], sem_xb.at[i])

        WA = 128 if SPLIT_A else D

        def cp_oa(i, n):
            return pltpu.make_async_copy(out_scr.at[pl.ds(i * T2, T2), pl.ds(n * WA, WA)],
                                         out_hbm.at[pl.ds(i * T2, T2), pl.ds(n * WA, WA)], sem_oa.at[i])

        WB = 128 if SPLIT_B else D

        RB = T2 // YROWS

        def cp_ob(i, n, m):
            return pltpu.make_async_copy(out_scr.at[pl.ds(i * T2 + m * RB, RB), pl.ds(D + n * WB, WB)],
                                         out_hbm.at[pl.ds(i * T2 + m * RB, RB), pl.ds(D + n * WB, WB)], sem_ob.at[i])

        c_wphi = cp_w(wphi_hbm, wphi, 0)
        c_wkv = cp_w(wqkv_hbm.at[:, pl.ds(D, 2 * D)], wkv, 1)
        c_wq = cp_w(wqkv_hbm.at[:, pl.ds(0, D)], wq, 3)
        c_lre = cp_w(lre_hbm, lre, 4)
        c_lim = cp_w(lim_hbm, lim, 5)
        c_ldt = cp_w(ldt_hbm, ldt, 6)
        c_dsk = cp_w(dsk_hbm, dsk, 7)
        c_cre = cp_w(cre_hbm, cre, 8)
        c_cim = cp_w(cim_hbm, cim, 9)
        c_bre = cp_w(bre_hbm, bre, 10)
        c_bim = cp_w(bim_hbm, bim, 11)
        c_wo = cp_w(wo_hbm, wo, 12)

        scope("S_mbuild")
        if XFIRST:
            c_wphi.start()
            cp_xa(0).start()
            c_wkv.start()
        else:
            c_wphi.start()
            c_wkv.start()
            cp_xa(0).start()

        c_wphi.wait()
        eye = (lax.broadcasted_iota(jnp.int32, (H, H), 0) == lax.broadcasted_iota(jnp.int32, (H, H), 1)).astype(BF16)
        lane_ok = lax.broadcasted_iota(jnp.int32, (H, 128), 1) < DH
        for i in range(DH):
            t_i = lax.dot_general(eye, wphi[i], NT, preferred_element_type=F32)
            t_i = jnp.where(lane_ok, jnp.pad(t_i, ((0, 0), (0, 128 - DH))), 0.0)
            r_scr[pl.ds(i, H, stride=DH), :] = t_i
        rr = _iota((160, 128), 0)
        cc = _iota((160, 128), 1)
        e_t = (_fdiv(rr - 40.0 * _fdiv(rr, 40), 2) == cc).astype(BF16)
        hrow = 2.0 * _fdiv(rr, 40) + (rr - 2.0 * _fdiv(rr, 2))
        for j in range(NC):
            rj = r_scr[pl.ds(128 * j, 128), :].astype(BF16)
            full = lax.dot_general(e_t, rj, NT, preferred_element_type=F32)
            mask = (hrow + 6.0 * j) == _fdiv(cc + 128.0 * j, DH)
            m_scr[j] = jnp.where(mask, full, 0.0).astype(BF16)

        def ssm_prep():

            def v5(ref):
                v = ref[...].astype(F32).reshape(1, D)
                return jnp.concatenate([v[:, 128 * c:128 * c + 128] for c in range(NC)], axis=0)

            l_re, l_im = v5(lre), v5(lim)
            dt = jnp.exp(v5(ldt)).astype(BF16).astype(F32)
            mag = jnp.exp(dt * l_re)
            ang = dt * l_im
            lb_re, lb_im = mag * jnp.cos(ang), mag * jnp.sin(ang)
            inv = 1.0 / (l_re * l_re + l_im * l_im)
            nr = lb_re - 1.0
            co_re = 2.0 * (nr * l_re + lb_im * l_im) * inv
            co_im = -2.0 * (lb_im * l_re - nr * l_im) * inv
            lam[pl.ds(0, NC), :] = lb_re
            lam[pl.ds(8, NC), :] = -lb_im
            dsk5 = v5(dsk)
            for c in range(NC):
                coef[0, :, pl.ds(128 * c, 128)] = jnp.broadcast_to(co_re[c:c + 1], (8, 128))
                coef[1, :, pl.ds(128 * c, 128)] = jnp.broadcast_to(co_im[c:c + 1], (8, 128))
                coef[2, :, pl.ds(128 * c, 128)] = jnp.broadcast_to(dsk5[c:c + 1], (8, 128))
        kvacc[...] = jnp.zeros(kvacc.shape, F32)

        def fold_rows(w_ref, c0):
            blks = [lax.dot_general(m_scr[j], w_ref[:, pl.ds(c0 + 128 * j, 128)], NT, preferred_element_type=F32)
                    for j in range(NC)]
            parts = [blks[0][0:120]]
            for j in range(1, NC):
                parts.append(blks[j - 1][120:160] + blks[j][0:40])
                parts.append(blks[j][40:120])
            parts.append(blks[NC - 1][120:160])
            return (jnp.concatenate(parts, axis=0) * LOG2E).astype(BF16)

        scope("S_foldk")
        c_wkv.wait()
        for i in range(1, N1):
            cp_xa(i).start()
        later = [c_lre, c_lim, c_ldt, c_dsk, c_wq, c_bre, c_bim, c_cre, c_cim, c_wo] + [cp_xb(i) for i in range(N2)]
        for c in later:
            c.start()
        wkT[...] = fold_rows(wkv, 0)
        wvT[...] = wkv[:, pl.ds(D, D)].T

        scope("S_phase1")

        def phase1(i, carry):
            cp_xa(i).wait()
            x = xa[pl.ds(_mo(i * T1, T1), T1), :]
            kT = lax.dot_general(wkT[...], x, NT, preferred_element_type=F32)
            w_v = wvT[...]
            vT = lax.dot_general(w_v, x, NT, preferred_element_type=F32)
            ones = jnp.ones((8, T1), F32)
            for g in range(NG):
                phi = _dual_softmax(kT[GR * g:GR * g + GR])
                vext = jnp.concatenate([vT[GR * g:GR * g + GR], ones], axis=0).astype(BF16)
                kvacc[g] += lax.dot_general(vext, phi, NT, preferred_element_type=F32)
            return carry

        lax.fori_loop(0, N1, phase1, 0)

        scope("S_trans")
        c_lre.wait(); c_lim.wait(); c_ldt.wait(); c_dsk.wait()
        c_wq.wait(); c_cre.wait(); c_cim.wait(); c_bre.wait(); c_bim.wait(); c_wo.wait()
        for i in range(N2):
            cp_xb(i).wait()
        wqT[...] = fold_rows(wq, 0)
        ssm_prep()
        r48 = _iota((48, 2 * GR), 0)
        c80 = _iota((48, 2 * GR), 1)
        head_r = jnp.where(r48 < 40.0, _fdiv(r48, DH), _fdiv(r48 - 40.0, 4))
        kvmask = head_r == (c80 - 2.0 * _fdiv(c80, 2))
        for g in range(NG):
            kvm[g] = jnp.where(kvmask, kvacc[g], 0.0).astype(BF16)

        scope("S_phase2")

        def phase2(i, carry):
            r0 = _mo(i * T2, T2)
            st = {"s": carry}
            x_b = xb[pl.ds(r0, T2), :]

            def op_ure():
                st["ure"] = lax.dot_general(x_b, bre[...], NT, preferred_element_type=F32)

            def op_uim():
                u_im = lax.dot_general(x_b, bim[...], NT, preferred_element_type=F32)
                u_re = st["ure"]
                for c in range(NC):
                    cols = pl.ds(128 * c, 128)
                    k_re = jnp.concatenate([coef[0, :, cols]] * (T2 // 8), axis=0)
                    k_im = jnp.concatenate([coef[1, :, cols]] * (T2 // 8), axis=0)
                    a, b = u_re[:, 128 * c:128 * c + 128], u_im[:, 128 * c:128 * c + 128]
                    ur[pl.ds(c * TS, T2), :] = k_re * a + k_im * b
                    ui[pl.ds(c * TS, T2), :] = k_im * a - k_re * b

            def op_pq():
                st["pq"] = lax.dot_general(wqT[...], xa[pl.ds(r0, T2), :], NT, preferred_element_type=F32)

            def op_scan():
                s_re, s_im = st["s"]
                lam_r, lam_i = lam[pl.ds(0, NC), :], lam[pl.ds(8, NC), :]
                for t in range(0, T2, 2):
                    a0, b0 = ur[pl.ds(t, NC, stride=TS), :], ui[pl.ds(t, NC, stride=TS), :]
                    a1, b1 = ur[pl.ds(t + 1, NC, stride=TS), :], ui[pl.ds(t + 1, NC, stride=TS), :]
                    p_re = lam_r * s_re - lam_i * s_im + a0
                    p_im = lam_r * s_im + lam_i * s_re + b0
                    s_re = lam_r * p_re - lam_i * p_im + a1
                    s_im = lam_r * p_im + lam_i * p_re + b1
                    hr[pl.ds(t // 2, NC, stride=TSH), :] = pltpu.pack_elementwise([p_re, s_re], packed_dtype=BF16)
                    hi[pl.ds(t // 2, NC, stride=TSH), :] = pltpu.pack_elementwise([p_im, s_im], packed_dtype=BF16)
                st["s"] = (s_re, s_im)

            def h_load(ref):
                return jnp.concatenate(
                    [pltpu.bitcast(ref[pl.ds(c * TSH, T2 // 2), :], BF16) for c in range(NC)], axis=1)

            def op_y():
                h_re, h_im = h_load(hr), h_load(hi)
                for m in range(YROWS):
                    rows = slice(m * RB, (m + 1) * RB)
                    for n in range(D // WB):
                        cols = pl.ds(n * WB, WB)
                        y = lax.dot_general(h_re[rows], cre[cols, :], NT, preferred_element_type=F32)
                        y = y + lax.dot_general(h_im[rows], cim[cols, :], NT, preferred_element_type=F32)
                        dskip = jnp.concatenate([coef[2, :, cols]] * (RB // 8), axis=0)
                        out_scr[pl.ds(r0 + m * RB, RB), pl.ds(D + n * WB, WB)] = (
                            y + x_b[rows, n * WB:(n + 1) * WB].astype(F32) * dskip)
                        cp_ob(i, n, m).start()

            def op_soft():
                pq = st["pq"]
                st["phi"] = [_dual_softmax(pq[GR * g:GR * g + GR]) for g in range(NG)]

            def op_num():
                low = lax.broadcasted_iota(jnp.int32, (8, T2), 0) < 4
                outs = []
                for g in range(NG):
                    nd = jnp.dot(kvm[g], st["phi"][g], preferred_element_type=F32)
                    r = _rcp(nd[40:48] + 1e-6)
                    rs = pltpu.roll(r, 4, 0)
                    ra, rb = jnp.where(low, r, rs), jnp.where(low, rs, r)
                    outs += [nd[0:8] * ra, nd[8:16] * ra, nd[16:24] * r, nd[24:32] * rb, nd[32:40] * rb]
                st["o"] = jnp.concatenate(outs, axis=0).astype(BF16).T

            def op_wo():
                o = st["o"]
                for n in range(D // WA):
                    out_scr[pl.ds(r0, T2), pl.ds(n * WA, WA)] = jnp.dot(
                        o, wo[:, pl.ds(n * WA, WA)], preferred_element_type=F32)
                    cp_oa(i, n).start()

            ops = dict(ure=op_ure, uim=op_uim, pq=op_pq, scan=op_scan, y=op_y,
                       soft=op_soft, num=op_num, wo=op_wo)
            for name in ORDER.split():
                ops[name]()
            return st["s"]

        z = jnp.zeros((NC, 128), F32)
        if N2 == 1:
            phase2(0, (z, z))
        else:
            lax.fori_loop(0, N2, phase2, (z, z))
        scope("S_tail")
        for i in range(N2):
            for n in range(D // WA):
                cp_oa(i, n).wait()
            for m in range(YROWS):
                for n in range(D // WB):
                    cp_ob(i, n, m).wait()
        scope(None)

    return kernel, N1, N2, TS, TSH


@jax.jit
def pallas_concat_heads__linear_kernel_hedgehog__ssm_conv_s5__prompt_kernel(
    A_x: jax.Array,
    A_wqkv: jax.Array,
    A_w_phi: jax.Array,
    A_wo: jax.Array,
    B_x: jax.Array,
    B_Lambda_re: jax.Array,
    B_Lambda_im: jax.Array,
    B_B_re: jax.Array,
    B_B_im: jax.Array,
    B_C_re: jax.Array,
    B_C_im: jax.Array,
    B_log_dt: jax.Array,
    B_Dskip: jax.Array,
):
    T1 = 512
    T2 = 1024
    ORDER = "pq ure soft num uim scan wo y"
    SPLIT_A = False
    SPLIT_B = True
    XFIRST = False
    YROWS = 2
    SCOPES = False
    kernel, N1, N2, TS, TSH = _make_kernel(T1, T2, ORDER, SPLIT_A, SPLIT_B, XFIRST, YROWS, SCOPES)
    any_spec = pl.BlockSpec(memory_space=pl.ANY)
    V = pltpu.VMEM
    scratch = [
        V((SEQ, D), BF16), V((SEQ, D), BF16),
        V((D, D), BF16), V((D, 2 * D), BF16), V((D, D), BF16),
        V((D, D), BF16), V((D, D), BF16), V((D, D), BF16), V((D, D), BF16),
        V((DH, DH, H), BF16), V((D,), BF16), V((D,), BF16), V((D,), BF16), V((D,), BF16),
        V((D, 128), F32), V((NC, 160, 128), BF16), V((D, D), BF16), V((D, D), BF16), V((D, D), BF16),
        V((NG, 48, 2 * GR), F32), V((NG, 48, 2 * GR), BF16),
        V((3, 8, D), F32), V((16, 128), F32),
        V((NC * TS + 4, 128), F32), V((NC * TS + 4, 128), F32),
        V((NC * TSH + 4, 128), jnp.int32), V((NC * TSH + 4, 128), jnp.int32),
        V((SEQ, 2 * D), F32),
        pltpu.SemaphoreType.DMA((13,)), pltpu.SemaphoreType.DMA((N1,)), pltpu.SemaphoreType.DMA((N2,)),
        pltpu.SemaphoreType.DMA((N2,)), pltpu.SemaphoreType.DMA((N2,)),
    ]
    out = pl.pallas_call(
        kernel,
        out_shape=jax.ShapeDtypeStruct((SEQ, 2 * D), F32),
        in_specs=[any_spec] * 13,
        out_specs=any_spec,
        scratch_shapes=scratch,
        compiler_params=pltpu.CompilerParams(vmem_limit_bytes=100 * 1024 * 1024),
        name="hedgehog_s5",
    )(A_x.reshape(SEQ, D), A_wqkv, jnp.transpose(A_w_phi, (1, 2, 0)), A_wo, B_x.reshape(SEQ, D),
      B_Lambda_re, B_Lambda_im, B_B_re, B_B_im, B_C_re, B_C_im, B_log_dt, B_Dskip)
    return out.reshape(1, SEQ, 2 * D)
```

```python
import numpy as np
import jax
import jax.numpy as jnp
from jax import lax
import jax.experimental.pallas as pl
import jax.experimental.pallas.tpu as pltpu

SEQ, D, H, DH = 2048, 640, 32, 20
NG = H // 2
GR = 2 * DH
NC = D // 128
T1, T2 = 512, 1024
N1, N2 = SEQ // T1, SEQ // T2
TS = T2 + 4
TSH = T2 // 2 + 4
RB = 128
LOG2E = float(np.log2(np.e))
F32, BF16 = jnp.float32, jnp.bfloat16
NT = (((1,), (1,)), ((), ()))


def _rcp(x):
    r = pltpu.reciprocal(x, approx=True)
    return r * (2.0 - x * r)


def _fdiv(x, n):
    return jnp.floor((x + 0.5) * (1.0 / n))


def _iota(shape, d):
    return lax.broadcasted_iota(jnp.int32, shape, d).astype(F32)


def _dual_softmax(p):
    pj = [p[8 * j:8 * j + 8] for j in range(5)]

    def allred(xs, op):
        m = op(op(op(xs[0], xs[1]), op(xs[2], xs[3])), xs[4])
        m = op(m, pltpu.roll(m, 4, 0))
        return op(m, pltpu.roll(m, 2, 0))

    mx = allred(pj, jnp.maximum)
    mn = allred(pj, jnp.minimum)
    ep = [jnp.exp2(x - mx) for x in pj]
    en = [jnp.exp2(mn - x) for x in pj]
    rp = _rcp(allred(ep, jnp.add))
    rn = _rcp(allred(en, jnp.add))
    return jnp.concatenate([e * rp for e in ep] + [e * rn for e in en], axis=0).astype(BF16)


def _kernel(ax_hbm, wqkv_hbm, wphi_hbm, wo_hbm, bx_hbm, lre_hbm, lim_hbm, bre_hbm, bim_hbm,
            cre_hbm, cim_hbm, ldt_hbm, dsk_hbm, out_hbm,
            xa, xb, wq, wkv, wo, bre, bim, cre, cim, wphi, lre, lim, ldt, dsk,
            r_scr, m_scr, wkT, wvT, wqT, kvacc, kvm, coef, lam, ur, ui, hr, hi, out_scr,
            sem_w, sem_xa, sem_xb, sem_oa, sem_ob):
    def cp_w(src, dst, k):
        return pltpu.make_async_copy(src, dst, sem_w.at[k])

    def cp_xa(i):
        return pltpu.make_async_copy(ax_hbm.at[pl.ds(i * T1, T1), :], xa.at[pl.ds(i * T1, T1), :], sem_xa.at[i])

    def cp_xb(i):
        return pltpu.make_async_copy(bx_hbm.at[pl.ds(i * T2, T2), :], xb.at[pl.ds(i * T2, T2), :], sem_xb.at[i])

    def cp_oa(i):
        return pltpu.make_async_copy(out_scr.at[pl.ds(i * T2, T2), pl.ds(0, D)],
                                     out_hbm.at[pl.ds(i * T2, T2), pl.ds(0, D)], sem_oa.at[i])

    def cp_ob(i, n, m):
        rows, cols = pl.ds(i * T2 + m * RB, RB), pl.ds(D + n * 128, 128)
        return pltpu.make_async_copy(out_scr.at[rows, cols], out_hbm.at[rows, cols], sem_ob.at[i])

    c_wphi = cp_w(wphi_hbm, wphi, 0)
    c_wkv = cp_w(wqkv_hbm.at[:, pl.ds(D, 2 * D)], wkv, 1)
    c_wq = cp_w(wqkv_hbm.at[:, pl.ds(0, D)], wq, 2)
    c_lre = cp_w(lre_hbm, lre, 3)
    c_lim = cp_w(lim_hbm, lim, 4)
    c_ldt = cp_w(ldt_hbm, ldt, 5)
    c_dsk = cp_w(dsk_hbm, dsk, 6)
    c_cre = cp_w(cre_hbm, cre, 7)
    c_cim = cp_w(cim_hbm, cim, 8)
    c_bre = cp_w(bre_hbm, bre, 9)
    c_bim = cp_w(bim_hbm, bim, 10)
    c_wo = cp_w(wo_hbm, wo, 11)

    c_wphi.start()
    c_wkv.start()
    cp_xa(0).start()

    c_wphi.wait()
    eye = (lax.broadcasted_iota(jnp.int32, (H, H), 0) == lax.broadcasted_iota(jnp.int32, (H, H), 1)).astype(BF16)
    lane_ok = lax.broadcasted_iota(jnp.int32, (H, 128), 1) < DH
    for i in range(DH):
        t_i = lax.dot_general(eye, wphi[i], NT, preferred_element_type=F32)
        t_i = jnp.where(lane_ok, jnp.pad(t_i, ((0, 0), (0, 128 - DH))), 0.0)
        r_scr[pl.ds(i, H, stride=DH), :] = t_i
    rr = _iota((160, 128), 0)
    cc = _iota((160, 128), 1)
    e_t = (_fdiv(rr - 40.0 * _fdiv(rr, 40), 2) == cc).astype(BF16)
    hrow = 2.0 * _fdiv(rr, 40) + (rr - 2.0 * _fdiv(rr, 2))
    for j in range(NC):
        rj = r_scr[pl.ds(128 * j, 128), :].astype(BF16)
        full = lax.dot_general(e_t, rj, NT, preferred_element_type=F32)
        mask = (hrow + 6.0 * j) == _fdiv(cc + 128.0 * j, DH)
        m_scr[j] = jnp.where(mask, full, 0.0).astype(BF16)
    kvacc[...] = jnp.zeros(kvacc.shape, F32)

    def fold(w_ref):
        blks = [lax.dot_general(m_scr[j], w_ref[:, pl.ds(128 * j, 128)], NT, preferred_element_type=F32)
                for j in range(NC)]
        parts = [blks[0][0:120]]
        for j in range(1, NC):
            parts.append(blks[j - 1][120:160] + blks[j][0:40])
            parts.append(blks[j][40:120])
        parts.append(blks[NC - 1][120:160])
        return (jnp.concatenate(parts, axis=0) * LOG2E).astype(BF16)

    c_wkv.wait()
    for i in range(1, N1):
        cp_xa(i).start()
    for c in [c_lre, c_lim, c_ldt, c_dsk, c_wq, c_bre, c_bim, c_cre, c_cim, c_wo] + [cp_xb(i) for i in range(N2)]:
        c.start()
    wkT[...] = fold(wkv)
    wvT[...] = wkv[:, pl.ds(D, D)].T

    def phase1(i, carry):
        cp_xa(i).wait()
        x = xa[pl.ds(pl.multiple_of(i * T1, T1), T1), :]
        kT = lax.dot_general(wkT[...], x, NT, preferred_element_type=F32)
        vT = lax.dot_general(wvT[...], x, NT, preferred_element_type=F32)
        ones = jnp.ones((8, T1), F32)
        for g in range(NG):
            phi = _dual_softmax(kT[GR * g:GR * g + GR])
            vext = jnp.concatenate([vT[GR * g:GR * g + GR], ones], axis=0).astype(BF16)
            kvacc[g] += lax.dot_general(vext, phi, NT, preferred_element_type=F32)
        return carry

    lax.fori_loop(0, N1, phase1, 0)

    c_lre.wait(); c_lim.wait(); c_ldt.wait(); c_dsk.wait()
    c_wq.wait(); c_cre.wait(); c_cim.wait(); c_bre.wait(); c_bim.wait(); c_wo.wait()
    for i in range(N2):
        cp_xb(i).wait()
    wqT[...] = fold(wq)

    def v5(ref):
        v = ref[...].astype(F32).reshape(1, D)
        return jnp.concatenate([v[:, 128 * c:128 * c + 128] for c in range(NC)], axis=0)

    l_re, l_im = v5(lre), v5(lim)
    dt = jnp.exp(v5(ldt)).astype(BF16).astype(F32)
    mag = jnp.exp(dt * l_re)
    ang = dt * l_im
    lb_re, lb_im = mag * jnp.cos(ang), mag * jnp.sin(ang)
    inv = 1.0 / (l_re * l_re + l_im * l_im)
    nr = lb_re - 1.0
    co_re = 2.0 * (nr * l_re + lb_im * l_im) * inv
    co_im = -2.0 * (lb_im * l_re - nr * l_im) * inv
    lam[pl.ds(0, NC), :] = lb_re
    lam[pl.ds(8, NC), :] = -lb_im
    dsk5 = v5(dsk)
    for c in range(NC):
        coef[0, :, pl.ds(128 * c, 128)] = jnp.broadcast_to(co_re[c:c + 1], (8, 128))
        coef[1, :, pl.ds(128 * c, 128)] = jnp.broadcast_to(co_im[c:c + 1], (8, 128))
        coef[2, :, pl.ds(128 * c, 128)] = jnp.broadcast_to(dsk5[c:c + 1], (8, 128))

    r48 = _iota((48, 2 * GR), 0)
    c80 = _iota((48, 2 * GR), 1)
    head_r = jnp.where(r48 < 40.0, _fdiv(r48, DH), _fdiv(r48 - 40.0, 4))
    kvmask = head_r == (c80 - 2.0 * _fdiv(c80, 2))
    for g in range(NG):
        kvm[g] = jnp.where(kvmask, kvacc[g], 0.0).astype(BF16)

    def phase2(i, carry):
        s_re, s_im = carry
        r0 = pl.multiple_of(i * T2, T2)
        x_b = xb[pl.ds(r0, T2), :]

        pq = lax.dot_general(wqT[...], xa[pl.ds(r0, T2), :], NT, preferred_element_type=F32)
        u_re = lax.dot_general(x_b, bre[...], NT, preferred_element_type=F32)
        phis = [_dual_softmax(pq[GR * g:GR * g + GR]) for g in range(NG)]

        low = lax.broadcasted_iota(jnp.int32, (8, T2), 0) < 4
        outs = []
        for g in range(NG):
            nd = jnp.dot(kvm[g], phis[g], preferred_element_type=F32)
            r = _rcp(nd[40:48] + 1e-6)
            rs = pltpu.roll(r, 4, 0)
            ra, rb = jnp.where(low, r, rs), jnp.where(low, rs, r)
            outs += [nd[0:8] * ra, nd[8:16] * ra, nd[16:24] * r, nd[24:32] * rb, nd[32:40] * rb]
        o = jnp.concatenate(outs, axis=0).astype(BF16).T

        u_im = lax.dot_general(x_b, bim[...], NT, preferred_element_type=F32)
        for c in range(NC):
            cols = pl.ds(128 * c, 128)
            k_re = jnp.concatenate([coef[0, :, cols]] * (T2 // 8), axis=0)
            k_im = jnp.concatenate([coef[1, :, cols]] * (T2 // 8), axis=0)
            a, b = u_re[:, 128 * c:128 * c + 128], u_im[:, 128 * c:128 * c + 128]
            ur[pl.ds(c * TS, T2), :] = k_re * a + k_im * b
            ui[pl.ds(c * TS, T2), :] = k_im * a - k_re * b

        lam_r, lam_i = lam[pl.ds(0, NC), :], lam[pl.ds(8, NC), :]
        for t in range(0, T2, 2):
            a0, b0 = ur[pl.ds(t, NC, stride=TS), :], ui[pl.ds(t, NC, stride=TS), :]
            a1, b1 = ur[pl.ds(t + 1, NC, stride=TS), :], ui[pl.ds(t + 1, NC, stride=TS), :]
            p_re = lam_r * s_re - lam_i * s_im + a0
            p_im = lam_r * s_im + lam_i * s_re + b0
            s_re = lam_r * p_re - lam_i * p_im + a1
            s_im = lam_r * p_im + lam_i * p_re + b1
            hr[pl.ds(t // 2, NC, stride=TSH), :] = pltpu.pack_elementwise([p_re, s_re], packed_dtype=BF16)
            hi[pl.ds(t // 2, NC, stride=TSH), :] = pltpu.pack_elementwise([p_im, s_im], packed_dtype=BF16)

        out_scr[pl.ds(r0, T2), pl.ds(0, D)] = jnp.dot(o, wo[...], preferred_element_type=F32)
        cp_oa(i).start()

        def h_load(ref):
            return jnp.concatenate(
                [pltpu.bitcast(ref[pl.ds(c * TSH, T2 // 2), :], BF16) for c in range(NC)], axis=1)

        h_re, h_im = h_load(hr), h_load(hi)
        for m in range(T2 // RB):
            rows = slice(m * RB, (m + 1) * RB)
            for n in range(NC):
                cols = pl.ds(n * 128, 128)
                y = lax.dot_general(h_re[rows], cre[cols, :], NT, preferred_element_type=F32)
                y = y + lax.dot_general(h_im[rows], cim[cols, :], NT, preferred_element_type=F32)
                dskip = jnp.concatenate([coef[2, :, cols]] * (RB // 8), axis=0)
                out_scr[pl.ds(r0 + m * RB, RB), pl.ds(D + n * 128, 128)] = (
                    y + x_b[rows, n * 128:(n + 1) * 128].astype(F32) * dskip)
                cp_ob(i, n, m).start()
        return s_re, s_im

    z = jnp.zeros((NC, 128), F32)
    lax.fori_loop(0, N2, phase2, (z, z))

    for i in range(N2):
        cp_oa(i).wait()
        for m in range(T2 // RB):
            for n in range(NC):
                cp_ob(i, n, m).wait()


@jax.jit
def pallas_concat_heads__linear_kernel_hedgehog__ssm_conv_s5__prompt_kernel(
    A_x: jax.Array,
    A_wqkv: jax.Array,
    A_w_phi: jax.Array,
    A_wo: jax.Array,
    B_x: jax.Array,
    B_Lambda_re: jax.Array,
    B_Lambda_im: jax.Array,
    B_B_re: jax.Array,
    B_B_im: jax.Array,
    B_C_re: jax.Array,
    B_C_im: jax.Array,
    B_log_dt: jax.Array,
    B_Dskip: jax.Array,
):
    any_spec = pl.BlockSpec(memory_space=pl.ANY)
    V = pltpu.VMEM
    mat = V((D, D), BF16)
    vec = V((D,), BF16)
    scratch = [
        V((SEQ, D), BF16), V((SEQ, D), BF16),
        mat, V((D, 2 * D), BF16), mat, mat, mat, mat, mat,
        V((DH, DH, H), BF16), vec, vec, vec, vec,
        V((D, 128), F32), V((NC, 160, 128), BF16), mat, mat, mat,
        V((NG, 48, 2 * GR), F32), V((NG, 48, 2 * GR), BF16),
        V((3, 8, D), F32), V((16, 128), F32),
        V((NC * TS + 4, 128), F32), V((NC * TS + 4, 128), F32),
        V((NC * TSH + 4, 128), jnp.int32), V((NC * TSH + 4, 128), jnp.int32),
        V((SEQ, 2 * D), F32),
        pltpu.SemaphoreType.DMA((12,)), pltpu.SemaphoreType.DMA((N1,)), pltpu.SemaphoreType.DMA((N2,)),
        pltpu.SemaphoreType.DMA((N2,)), pltpu.SemaphoreType.DMA((N2,)),
    ]
    out = pl.pallas_call(
        _kernel,
        out_shape=jax.ShapeDtypeStruct((SEQ, 2 * D), F32),
        in_specs=[any_spec] * 13,
        out_specs=any_spec,
        scratch_shapes=scratch,
        compiler_params=pltpu.CompilerParams(vmem_limit_bytes=100 * 1024 * 1024),
        name="hedgehog_s5",
    )(A_x.reshape(SEQ, D), A_wqkv, jnp.transpose(A_w_phi, (1, 2, 0)), A_wo, B_x.reshape(SEQ, D),
      B_Lambda_re, B_Lambda_im, B_B_re, B_B_im, B_C_re, B_C_im, B_log_dt, B_Dskip)
    return out.reshape(1, SEQ, 2 * D)
```
